```python
import jax
import jax.numpy as jnp

def _softmax(x, axis=-1):
    return jax.nn.softmax(x, axis=axis)
def _gelu(x):
    return jax.nn.gelu(x, approximate=True)
def _silu(x):
    return jax.nn.silu(x)
def _sigmoid(x):
    return jax.nn.sigmoid(x)
def _layernorm(x, axis=-1, eps=1e-5):
    m = jnp.mean(x, axis=axis, keepdims=True)
    v = jnp.var(x, axis=axis, keepdims=True)
    return (x - m) / jnp.sqrt(v + eps)
def _scatter_add(tgt, idx, src, axis=0):
    return tgt.at[idx].add(src)
def _segment_sum(src, seg, n):
    return jax.ops.segment_sum(src, seg, n)
class _Rng:
    def __init__(self, key):
        self._k = key
    def _next(self):
        self._k, sub = jax.random.split(self._k)
        return sub
    def normal(self, shape):
        return jax.random.normal(self._next(), shape, dtype=jnp.bfloat16)
    def randint(self, lo, hi, shape):
        return jax.random.randint(self._next(), shape, lo, hi, dtype=jnp.int32)
    def uniform(self, shape, lo=0.0, hi=1.0):
        return jax.random.uniform(self._next(), shape, jnp.bfloat16, lo, hi)
    def permutation(self, n):
        return jax.random.permutation(self._next(), n)


kernel_name = 'sequential_preLN__mha_block_cached__moe_arch_mod__decode'

def setup_inputs():
    _rng = _Rng(jax.random.key(int.from_bytes(__import__("os").urandom(4), "little")))
    _w = (lambda a: (lambda t: t.astype(jnp.bfloat16) if jnp.issubdtype(t.dtype, jnp.floating) else t)(jnp.asarray(a)))
    def _A_setup():
        B, Sq, D = 4, 1, 640
        H, Sk, Dh = 32, 8192, 192
        return {
            "x": _w((lambda *s: _rng.normal(s) * 0.05)(B, Sq, D)),
            "k_cache": _w((lambda *s: _rng.normal(s) * 0.05)(B, H, Sk, Dh)),
            "v_cache": _w((lambda *s: _rng.normal(s) * 0.05)(B, H, Sk, Dh)),
            "wq": _w((lambda *s: _rng.normal(s) * 0.05)(D, H * Dh) * (D ** -0.5)),
            "wo": _w((lambda *s: _rng.normal(s) * 0.05)(H * Dh, D) * ((H * Dh) ** -0.5)),
        }
    _A_in = _A_setup()

    def _B_setup():
        B, S, D, F, C = 4, 1, 640, 1536, 1
        return {
            "x": _w((lambda *s: _rng.normal(s) * 0.05)(B, S, D)),
            "w_r": _w((lambda *s: _rng.normal(s) * 0.05)(D)),
            "w_gate": _w((lambda *s: _rng.normal(s) * 0.05)(D, F)),
            "w_up": _w((lambda *s: _rng.normal(s) * 0.05)(D, F)),
            "w_down": _w((lambda *s: _rng.normal(s) * 0.05)(F, D)),
        }
    _B_in = _B_setup()

    return {
        "A_x": _A_in["x"],
        "A_k_cache": _A_in["k_cache"],
        "A_v_cache": _A_in["v_cache"],
        "A_wq": _A_in["wq"],
        "A_wo": _A_in["wo"],
        "B_x": _B_in["x"],
        "B_w_r": _B_in["w_r"],
        "B_w_gate": _B_in["w_gate"],
        "B_w_up": _B_in["w_up"],
        "B_w_down": _B_in["w_down"],
    }

def reference(A_x, A_k_cache, A_v_cache, A_wq, A_wo, B_x, B_w_r, B_w_gate, B_w_up, B_w_down):
    def _A_ref(x, k_cache, v_cache, wq, wo):
        B, Sq, D = x.shape
        H, Dh = 32, 192
        q = (lambda x, *d: x.transpose(*d))((x @ wq).reshape(B, Sq, H, Dh), 0, 2, 1, 3)
        scores = jnp.einsum("bhqd,bhkd->bhqk", q, k_cache) * (Dh ** -0.5)
        p = _softmax(scores, axis=-1)
        o = jnp.einsum("bhqk,bhkd->bhqd", p, v_cache)
        return (lambda x, *d: x.transpose(*d))(o, 0, 2, 1, 3).reshape(B, Sq, H * Dh) @ wo

    def _B_ref(x, w_r, w_gate, w_up, w_down):
        B, S, D = x.shape
        C = 1
        r = x @ w_r
        idx = jnp.argsort(-r, axis=-1)[:, :C]
        idx_e = jnp.repeat(idx.reshape(B, C, 1), D, axis=2)
        x_sel = jnp.take_along_axis(x, idx_e, axis=1)
        g = _silu(x_sel @ w_gate)
        u = x_sel @ w_up
        y = (g * u) @ w_down
        r_sel = _sigmoid(jnp.take_along_axis(r, idx, axis=1))
        y = y * r_sel.reshape(B, C, 1)
        b_off = (jnp.arange(B) * S).reshape(B, 1)
        flat_idx = (idx + b_off).reshape(B * C)
        zero = (x * 0.0).reshape(B * S, D)
        upd = _scatter_add(zero, flat_idx, y.reshape(B * C, D), axis=0)
        return x + upd.reshape(B, S, D)

    x = A_x
    h = x + _A_ref(_layernorm(x, axis=-1), A_k_cache, A_v_cache, A_wq, A_wo)
    h2 = h + _B_ref(_layernorm(h, axis=-1), B_w_r, B_w_gate, B_w_up, B_w_down)
    return h2
```

```python
import functools

import jax
import jax.numpy as jnp
from jax import lax
import jax.experimental.pallas as pl
import jax.experimental.pallas.tpu as pltpu

B, H, S, DH, D, F = 4, 32, 8192, 192, 640, 1536
NT = B * H
EPS = 1e-5
SCALE = DH ** -0.5

NK = 4
NV = 4
WK = 512
WV = 256

f32 = jnp.float32
bf16 = jnp.bfloat16


def _layernorm(x):
    m = jnp.mean(x, axis=-1, keepdims=True)
    c = x - m
    v = jnp.mean(c * c, axis=-1, keepdims=True)
    return c / jnp.sqrt(v + EPS)


def _kernel(x_ref, wr_ref, kt_hbm, vt_hbm, wq_hbm, wo_hbm, wg_hbm, wu_hbm, wd_hbm,
            out_ref,
            kbuf, vbuf, wq_v, wo_v, wg_v, wu_v, wd_v,
            q_scr, s_scr, attn_scr,
            ksem, vsem, wsem):

    def k_copy(t, slot):
        return pltpu.make_async_copy(kt_hbm.at[t], kbuf.at[slot], ksem.at[slot])

    def v_copy(t, slot):
        return pltpu.make_async_copy(vt_hbm.at[t], vbuf.at[slot], vsem.at[slot])

    wq_copy = pltpu.make_async_copy(wq_hbm, wq_v, wsem.at[0])
    wo_copy = pltpu.make_async_copy(wo_hbm, wo_v, wsem.at[1])
    wg_copy = pltpu.make_async_copy(wg_hbm, wg_v, wsem.at[2])
    wu_copy = pltpu.make_async_copy(wu_hbm, wu_v, wsem.at[3])
    wd_copy = pltpu.make_async_copy(wd_hbm, wd_v, wsem.at[4])

    wq_copy.start()
    k_copy(0, 0).start()
    wo_copy.start()
    v_copy(0, 0).start()
    for i in range(1, max(NK, NV)):
        if i < NK:
            k_copy(i, i).start()
        if i < NV:
            v_copy(i, i).start()
    wg_copy.start()
    wu_copy.start()
    wd_copy.start()

    x = x_ref[...].astype(f32)
    xn = _layernorm(x).astype(bf16)
    wq_copy.wait()
    q_all = jnp.dot(xn, wq_v[...], preferred_element_type=f32)
    q_all = q_all.astype(bf16).astype(f32) * SCALE
    for h in range(H):
        q_scr[h] = q_all[:, h * DH:(h + 1) * DH]
    attn_scr[...] = jnp.zeros(attn_scr.shape, f32)
    wo_copy.wait()

    row = lax.broadcasted_iota(jnp.int32, (DH, DH), 0)
    col = lax.broadcasted_iota(jnp.int32, (DH, DH), 1)
    eye = row == col

    def step(t, carry):
        b = t // H
        h = t % H
        kslot = t % NK
        vslot = t % NV

        qrow = q_scr[h, pl.ds(b, 1), :]
        qcol = jnp.sum(jnp.where(eye, qrow, 0.0), axis=1, keepdims=True)
        qb = jnp.broadcast_to(qcol, (DH, 128))

        k_copy(t, kslot).wait()

        def k_body(c, _):
            off = pl.multiple_of(c * WK, WK)
            for j in range(WK // 128):
                o2 = pl.multiple_of(off + j * 128, 128)
                kc = kbuf[kslot, :, pl.ds(o2, 128)].astype(f32)
                s_scr[:, pl.ds(o2, 128)] = jnp.sum(kc * qb, axis=0, keepdims=True)
            return 0

        lax.fori_loop(0, S // WK, k_body, 0)

        @pl.when(t + NK < NT)
        def _():
            k_copy(t + NK, kslot).start()

        s = s_scr[...]
        m = jnp.max(s, axis=1, keepdims=True)
        p = jnp.exp(s - m)
        l = jnp.sum(p, axis=1, keepdims=True)
        s_scr[...] = p

        v_copy(t, vslot).wait()

        def v_body(c, acc):
            off = pl.multiple_of(c * WV, WV)
            for j in range(WV // 128):
                o2 = pl.multiple_of(off + j * 128, 128)
                vc = vbuf[vslot, :, pl.ds(o2, 128)].astype(f32)
                acc = acc + vc * s_scr[:, pl.ds(o2, 128)]
            return acc

        acc = lax.fori_loop(0, S // WV, v_body, jnp.zeros((DH, 128), f32))

        @pl.when(t + NV < NT)
        def _():
            v_copy(t + NV, vslot).start()

        o = jnp.sum(acc, axis=1, keepdims=True) / l
        o = o.astype(bf16).astype(f32)
        wo_h = wo_v[pl.ds(pl.multiple_of(h * DH, 16), DH), :].astype(f32)
        contrib = (wo_h * o).reshape(DH // 8, 8, D).sum(axis=0)
        attn_scr[b] = attn_scr[b] + contrib
        return carry

    lax.fori_loop(0, NT, step, 0)

    attn = jnp.sum(attn_scr[...], axis=1)
    hres = x + attn
    hn = _layernorm(hres)
    hn16 = hn.astype(bf16)
    r = jnp.sum(hn16.astype(f32) * wr_ref[...].astype(f32), axis=1, keepdims=True)
    wg_copy.wait()
    wu_copy.wait()
    g = jnp.dot(hn16, wg_v[...], preferred_element_type=f32)
    u = jnp.dot(hn16, wu_v[...], preferred_element_type=f32)
    mid = (g * jax.nn.sigmoid(g) * u).astype(bf16)
    wd_copy.wait()
    y = jnp.dot(mid, wd_v[...], preferred_element_type=f32)
    y = y * jax.nn.sigmoid(r)
    out_ref[...] = (hres + (hn + y)).astype(out_ref.dtype)


@jax.jit
def pallas_sequential_preLN__mha_block_cached__moe_arch_mod__decode_kernel(
    A_x: jax.Array,
    A_k_cache: jax.Array,
    A_v_cache: jax.Array,
    A_wq: jax.Array,
    A_wo: jax.Array,
    B_x: jax.Array,
    B_w_r: jax.Array,
    B_w_gate: jax.Array,
    B_w_up: jax.Array,
    B_w_down: jax.Array,
):
    x2 = A_x.reshape(B, D)
    wr2 = B_w_r.reshape(1, D)
    kt = jnp.swapaxes(A_k_cache, 2, 3).reshape(NT, DH, S)
    vt = jnp.swapaxes(A_v_cache, 2, 3).reshape(NT, DH, S)

    any_spec = pl.BlockSpec(memory_space=pl.ANY)
    vmem_spec = pl.BlockSpec(memory_space=pltpu.VMEM)

    out = pl.pallas_call(
        _kernel,
        out_shape=jax.ShapeDtypeStruct((B, D), bf16),
        in_specs=[vmem_spec, vmem_spec] + [any_spec] * 7,
        out_specs=vmem_spec,
        scratch_shapes=[
            pltpu.VMEM((NK, DH, S), bf16),
            pltpu.VMEM((NV, DH, S), bf16),
            pltpu.VMEM((D, H * DH), bf16),
            pltpu.VMEM((H * DH, D), bf16),
            pltpu.VMEM((D, F), bf16),
            pltpu.VMEM((D, F), bf16),
            pltpu.VMEM((F, D), bf16),
            pltpu.VMEM((H, B, DH), f32),
            pltpu.VMEM((1, S), f32),
            pltpu.VMEM((B, 8, D), f32),
            pltpu.SemaphoreType.DMA((NK,)),
            pltpu.SemaphoreType.DMA((NV,)),
            pltpu.SemaphoreType.DMA((5,)),
        ],
        compiler_params=pltpu.CompilerParams(vmem_limit_bytes=100 * 1024 * 1024),
    )(x2, wr2, kt, vt, A_wq, A_wo, B_w_gate, B_w_up, B_w_down)
    return out.reshape(B, 1, D)
```

```python
import functools

import jax
import jax.numpy as jnp
from jax import lax
import jax.experimental.pallas as pl
import jax.experimental.pallas.tpu as pltpu

B, H, S, DH, D, F = 4, 32, 8192, 192, 640, 1536
NT = B * H
EPS = 1e-5
SCALE = DH ** -0.5

NB = 3
PC = 256
WK = 512
WV = 256
NPC = S // PC

f32 = jnp.float32
bf16 = jnp.bfloat16


def _layernorm(x):
    m = jnp.mean(x, axis=-1, keepdims=True)
    c = x - m
    v = jnp.mean(c * c, axis=-1, keepdims=True)
    return c / jnp.sqrt(v + EPS)


def _kernel(x_ref, wr_ref, kt_hbm, vt_hbm, wq_hbm, wo_hbm, wg_hbm, wu_hbm, wd_hbm,
            out_ref,
            kbuf, vbuf, wq_v, wo_v, wg_v, wu_v, wd_v,
            q_scr, s_scr, attn_scr,
            ksem, vsem, wsem):

    def piece(hbm, buf, sem, t, slot, off, prio):
        pltpu.make_async_copy(hbm.at[t, :, pl.ds(off, PC)], buf.at[slot, :, pl.ds(off, PC)],
                              sem.at[slot]).start(priority=prio)

    def issue_pair(t, slot, off):
        piece(kt_hbm, kbuf, ksem, t, slot, off, 0)
        piece(vt_hbm, vbuf, vsem, t, slot, off, 1)

    def slab_wait(buf, sem, slot):
        pltpu.make_async_copy(buf.at[slot], buf.at[slot], sem.at[slot]).wait()

    wq_copy = pltpu.make_async_copy(wq_hbm, wq_v, wsem.at[0])
    wo_copy = pltpu.make_async_copy(wo_hbm, wo_v, wsem.at[1])
    wg_copy = pltpu.make_async_copy(wg_hbm, wg_v, wsem.at[2])
    wu_copy = pltpu.make_async_copy(wu_hbm, wu_v, wsem.at[3])
    wd_copy = pltpu.make_async_copy(wd_hbm, wd_v, wsem.at[4])

    wq_copy.start()
    wo_copy.start(priority=1)
    for i in range(NB):
        def go(j, _):
            issue_pair(i, i, pl.multiple_of(j * PC, PC))
            return 0
        lax.fori_loop(0, NPC, go, 0)
    wg_copy.start()
    wu_copy.start(priority=1)
    wd_copy.start()

    x = x_ref[...].astype(f32)
    xn = _layernorm(x).astype(bf16)
    wq_copy.wait()
    q_all = jnp.dot(xn, wq_v[...], preferred_element_type=f32)
    q_all = q_all.astype(bf16).astype(f32) * SCALE
    for h in range(H):
        q_scr[h] = q_all[:, h * DH:(h + 1) * DH]
    attn_scr[...] = jnp.zeros(attn_scr.shape, f32)
    wo_copy.wait()

    row = lax.broadcasted_iota(jnp.int32, (DH, DH), 0)
    col = lax.broadcasted_iota(jnp.int32, (DH, DH), 1)
    eye = row == col

    def step(t, slot, prefetch):
        b = lax.shift_right_logical(t, 5)
        h = t & (H - 1)

        qrow = q_scr[h, pl.ds(b, 1), :]
        qcol = jnp.sum(jnp.where(eye, qrow, 0.0), axis=1, keepdims=True)
        qb = jnp.broadcast_to(qcol, (DH, 128))

        slab_wait(kbuf, ksem, slot)

        def k_body(c, _):
            off = pl.multiple_of(c * WK, WK)
            for j in range(WK // 256):
                o2 = pl.multiple_of(off + j * 256, 256)
                parts = [[None] * 2 for _ in range(2)]
                for r in range(DH // 8):
                    kc = kbuf[slot, r * 8:(r + 1) * 8, pl.ds(o2, 256)].astype(f32)
                    qr = qb[r * 8:(r + 1) * 8, :]
                    for hf in range(2):
                        pr = kc[:, hf * 128:(hf + 1) * 128] * qr
                        a = parts[hf][r % 2]
                        parts[hf][r % 2] = pr if a is None else a + pr
                for hf in range(2):
                    sv = parts[hf][0] + parts[hf][1]
                    s_scr[:, pl.ds(pl.multiple_of(o2 + hf * 128, 128), 128)] = jnp.sum(sv, axis=0, keepdims=True)
            return 0

        lax.fori_loop(0, S // WK, k_body, 0)

        s = s_scr[...]
        m = jnp.max(s, axis=1, keepdims=True)
        p = jnp.exp(s - m)
        l = jnp.sum(p, axis=1, keepdims=True)
        s_scr[...] = p

        slab_wait(vbuf, vsem, slot)

        def v_body(c, acc):
            off = pl.multiple_of(c * WV, WV)
            vc = vbuf[slot, :, pl.ds(off, WV)].astype(f32)
            for j in range(WV // 128):
                o2 = pl.multiple_of(off + j * 128, 128)
                acc = acc + vc[:, j * 128:(j + 1) * 128] * s_scr[:, pl.ds(o2, 128)]
            if prefetch:
                for j in range(WV // PC):
                    issue_pair(t + NB, slot, pl.multiple_of(off + j * PC, PC))
            return acc

        acc = lax.fori_loop(0, S // WV, v_body, jnp.zeros((DH, 128), f32))

        o = jnp.sum(acc, axis=1, keepdims=True) / l
        o = o.astype(bf16).astype(f32)
        wo_h = wo_v[pl.ds(pl.multiple_of(h * DH, 16), DH), :].astype(f32)
        contrib = (wo_h * o).reshape(DH // 8, 8, D).sum(axis=0)
        attn_scr[b] = attn_scr[b] + contrib

    def main_step(t, slot):
        step(t, slot, True)
        nslot = slot + 1
        return jnp.where(nslot == NB, 0, nslot)

    slot = lax.fori_loop(0, NT - NB, main_step, jnp.int32(0))

    def tail_step(t, slot):
        step(t, slot, False)
        nslot = slot + 1
        return jnp.where(nslot == NB, 0, nslot)

    lax.fori_loop(NT - NB, NT, tail_step, slot)

    attn = jnp.sum(attn_scr[...], axis=1)
    hres = x + attn
    hn = _layernorm(hres)
    hn16 = hn.astype(bf16)
    r = jnp.sum(hn16.astype(f32) * wr_ref[...].astype(f32), axis=1, keepdims=True)
    wg_copy.wait()
    wu_copy.wait()
    g = jnp.dot(hn16, wg_v[...], preferred_element_type=f32)
    u = jnp.dot(hn16, wu_v[...], preferred_element_type=f32)
    mid = (g * jax.nn.sigmoid(g) * u).astype(bf16)
    wd_copy.wait()
    y = jnp.dot(mid, wd_v[...], preferred_element_type=f32)
    y = y * jax.nn.sigmoid(r)
    out_ref[...] = (hres + (hn + y)).astype(out_ref.dtype)


@jax.jit
def pallas_sequential_preLN__mha_block_cached__moe_arch_mod__decode_kernel(
    A_x, A_k_cache, A_v_cache, A_wq, A_wo, B_x, B_w_r, B_w_gate, B_w_up, B_w_down,
):
    x2 = A_x.reshape(B, D)
    wr2 = B_w_r.reshape(1, D)
    kt = jnp.swapaxes(A_k_cache, 2, 3).reshape(NT, DH, S)
    vt = jnp.swapaxes(A_v_cache, 2, 3).reshape(NT, DH, S)

    any_spec = pl.BlockSpec(memory_space=pl.ANY)
    vmem_spec = pl.BlockSpec(memory_space=pltpu.VMEM)

    out = pl.pallas_call(
        _kernel,
        out_shape=jax.ShapeDtypeStruct((B, D), bf16),
        in_specs=[vmem_spec, vmem_spec] + [any_spec] * 7,
        out_specs=vmem_spec,
        scratch_shapes=[
            pltpu.VMEM((NB, DH, S), bf16),
            pltpu.VMEM((NB, DH, S), bf16),
            pltpu.VMEM((D, H * DH), bf16),
            pltpu.VMEM((H * DH, D), bf16),
            pltpu.VMEM((D, F), bf16),
            pltpu.VMEM((D, F), bf16),
            pltpu.VMEM((F, D), bf16),
            pltpu.VMEM((H, B, DH), f32),
            pltpu.VMEM((1, S), f32),
            pltpu.VMEM((B, 8, D), f32),
            pltpu.SemaphoreType.DMA((NB,)),
            pltpu.SemaphoreType.DMA((NB,)),
            pltpu.SemaphoreType.DMA((5,)),
        ],
        compiler_params=pltpu.CompilerParams(vmem_limit_bytes=100 * 1024 * 1024,
                                             disable_bounds_checks=True),
    )(x2, wr2, kt, vt, A_wq, A_wo, B_w_gate, B_w_up, B_w_down)
    return out.reshape(B, 1, D)
```

```python
import jax
import jax.numpy as jnp
from jax import lax
import jax.experimental.pallas as pl
import jax.experimental.pallas.tpu as pltpu

B, H, S, DH, D, F = 4, 32, 8192, 192, 640, 1536
NT = B * H
EPS = 1e-5
SCALE = DH ** -0.5

NB = 3
WK = 512
WV = 256
SPLIT = (24, 24, 16)
OFFS = [sum(SPLIT[:i]) * 128 for i in range(len(SPLIT))]
NROW = DH // 8
NWD = 3

f32 = jnp.float32
bf16 = jnp.bfloat16


def _layernorm(x):
    m = jnp.mean(x, axis=-1, keepdims=True)
    c = x - m
    v = jnp.mean(c * c, axis=-1, keepdims=True)
    return c / jnp.sqrt(v + EPS)


def _kernel(x_hbm, wr_hbm, kt_hbm, vt_hbm, wq_hbm, wo_hbm, wg_hbm, wu_hbm, wd_hbm,
            out_ref,
            kbuf, vbuf, x_v, wr_v, wq_v, wo_v, wg_v, wu_v, wd_v,
            q_scr, s_scr, attn_scr,
            ksem, vsem, wsem, dsem):

    def piece(hbm, buf, sem, t, slot, r, u, prio):
        w = SPLIT[u] * 128
        pltpu.make_async_copy(hbm.at[t, r, :, pl.ds(OFFS[u], w)], buf.at[slot, r, :, pl.ds(OFFS[u], w)],
                              sem.at[slot]).start(priority=prio)

    def issue(t, slot, r):
        n = len(SPLIT)
        for u in range(n):
            piece(kt_hbm, kbuf, ksem, t, slot, r, u, u % 2)
        for u in range(n):
            piece(vt_hbm, vbuf, vsem, t, slot, r, u, (n + u) % 2)

    def wait_all(buf, sem):
        pltpu.make_async_copy(buf, buf, sem).wait()

    def rows_piece(hbm, vm, sem, r0, nrows, prio):
        pltpu.make_async_copy(hbm.at[pl.ds(r0, nrows), :], vm.at[pl.ds(r0, nrows), :], sem).start(priority=prio)

    def wq_go(r, _):
        r0 = pl.multiple_of(r * 8, 8)
        for u in range(2):
            c0 = u * (H * DH // 2)
            pltpu.make_async_copy(wq_hbm.at[pl.ds(r0, 8), pl.ds(c0, H * DH // 2)],
                                  wq_v.at[pl.ds(r0, 8), pl.ds(c0, H * DH // 2)], wsem.at[0]).start(priority=u)
        return 0
    lax.fori_loop(0, D // 8, wq_go, 0)

    x_copy = pltpu.make_async_copy(x_hbm, x_v, wsem.at[4])
    wr_copy = pltpu.make_async_copy(wr_hbm, wr_v, wsem.at[5])
    x_copy.start()
    wr_copy.start(priority=1)

    for i in range(NB - 1):
        def go(j, _):
            issue(i, i, j)
            return 0
        lax.fori_loop(0, NROW, go, 0)

    def wo_go(r, _):
        for u in range(2):
            rows_piece(wo_hbm, wo_v, wsem.at[1], pl.multiple_of((2 * r + u) * 32, 32), 32, u)
        return 0
    lax.fori_loop(0, H * DH // 64, wo_go, 0)

    x_copy.wait()
    x = x_v[...].astype(f32)
    xn = _layernorm(x).astype(bf16)
    wait_all(wq_v, wsem.at[0])
    q_all = jnp.dot(xn, wq_v[...], preferred_element_type=f32)
    q_all = q_all.astype(bf16).astype(f32) * SCALE
    for h in range(H):
        q_scr[h] = q_all[:, h * DH:(h + 1) * DH]
    attn_scr[...] = jnp.zeros(attn_scr.shape, f32)
    wait_all(wo_v, wsem.at[1])

    row = lax.broadcasted_iota(jnp.int32, (DH, DH), 0)
    col = lax.broadcasted_iota(jnp.int32, (DH, DH), 1)
    eye = row == col

    def ffn_issue(c):
        @pl.when(c < 20)
        def _():
            r0 = pl.multiple_of(c * 32, 32)
            rows_piece(wg_hbm, wg_v, wsem.at[2], r0, 16, 0)
            rows_piece(wu_hbm, wu_v, wsem.at[3], r0, 16, 1)
            rows_piece(wg_hbm, wg_v, wsem.at[2], r0 + 16, 16, 0)
            rows_piece(wu_hbm, wu_v, wsem.at[3], r0 + 16, 16, 1)
        @pl.when(c >= 20)
        def _():
            cc = c - 20
            r0 = pl.multiple_of(cc * 128, 128)
            sem = dsem.at[lax.div(cc, jnp.int32(12 // NWD))]
            for u in range(4):
                rows_piece(wd_hbm, wd_v, sem, r0 + 32 * u, 32, u % 2)

    def step(t, slot, prefetch):
        b = lax.shift_right_logical(t, 5)
        h = t & (H - 1)
        pslot = jnp.where(slot == 0, NB - 1, slot - 1)

        qrow = q_scr[h, pl.ds(b, 1), :]
        qcol = jnp.sum(jnp.where(eye, qrow, 0.0), axis=1, keepdims=True)
        qb = jnp.broadcast_to(qcol, (DH, 128))

        wait_all(kbuf.at[slot], ksem.at[slot])

        def k_body(c, _):
            off = pl.multiple_of(c * WK, WK)
            for j in range(WK // 256):
                o2 = pl.multiple_of(off + j * 256, 256)
                parts = [[None] * 2 for _ in range(2)]
                for r in range(NROW):
                    kc = kbuf[slot, r, :, pl.ds(o2, 256)].astype(f32)
                    qr = qb[r * 8:(r + 1) * 8, :]
                    for hf in range(2):
                        pr = kc[:, hf * 128:(hf + 1) * 128] * qr
                        a = parts[hf][r % 2]
                        parts[hf][r % 2] = pr if a is None else a + pr
                for hf in range(2):
                    sv = parts[hf][0] + parts[hf][1]
                    s_scr[:, pl.ds(pl.multiple_of(o2 + hf * 128, 128), 128)] = jnp.sum(sv, axis=0, keepdims=True)
            return 0

        lax.fori_loop(0, S // WK, k_body, 0)

        s = s_scr[...]
        m = jnp.max(s, axis=1, keepdims=True)
        p = jnp.exp(s - m)
        l = jnp.sum(p, axis=1, keepdims=True)
        s_scr[...] = p

        wait_all(vbuf.at[slot], vsem.at[slot])

        def v_body(c, acc):
            off = pl.multiple_of(c * WV, WV)
            vc = vbuf[slot, :, :, pl.ds(off, WV)].astype(f32).reshape(DH, WV)
            for j in range(WV // 128):
                o2 = pl.multiple_of(off + j * 128, 128)
                acc = acc + vc[:, j * 128:(j + 1) * 128] * s_scr[:, pl.ds(o2, 128)]
            if prefetch == "kv":
                @pl.when(c < NROW)
                def _():
                    issue(t + NB - 1, pslot, c)
            elif prefetch == "ffn":
                ffn_issue(c)
            return acc

        acc = lax.fori_loop(0, S // WV, v_body, jnp.zeros((DH, 128), f32))

        o = jnp.sum(acc, axis=1, keepdims=True) / l
        o = o.astype(bf16).astype(f32)
        wo_h = wo_v[pl.ds(pl.multiple_of(h * DH, 16), DH), :].astype(f32)
        contrib = (wo_h * o).reshape(DH // 8, 8, D).sum(axis=0)
        attn_scr[b] = attn_scr[b] + contrib
        nslot = slot + 1
        return jnp.where(nslot == NB, 0, nslot)

    slot = lax.fori_loop(0, NT - NB + 1, lambda t, s: step(t, s, "kv"), jnp.int32(0))
    slot = step(jnp.int32(NT - NB + 1), slot, "ffn")
    lax.fori_loop(NT - NB + 2, NT, lambda t, s: step(t, s, None), slot)

    attn = jnp.sum(attn_scr[...], axis=1)
    hres = x + attn
    hn = _layernorm(hres)
    hn16 = hn.astype(bf16)
    wr_copy.wait()
    hnr = hn16.astype(f32)
    racc = hnr[:, 0:128] * wr_v[0:1, :].astype(f32)
    for i in range(1, D // 128):
        racc = racc + hnr[:, i * 128:(i + 1) * 128] * wr_v[i:i + 1, :].astype(f32)
    r = jnp.sum(racc, axis=1, keepdims=True)
    gate = jax.nn.sigmoid(r)
    base = hres + hn
    wait_all(wg_v, wsem.at[2])
    g = jnp.dot(hn16, wg_v[...], preferred_element_type=f32)
    wait_all(wu_v, wsem.at[3])
    u = jnp.dot(hn16, wu_v[...], preferred_element_type=f32)
    mid = (g * jax.nn.sigmoid(g) * u).astype(bf16)
    CH = F // NWD
    y = None
    for i in range(NWD):
        wait_all(wd_v.at[pl.ds(i * CH, CH), :], dsem.at[i])
        yi = jnp.dot(mid[:, i * CH:(i + 1) * CH], wd_v[i * CH:(i + 1) * CH, :], preferred_element_type=f32)
        y = yi if y is None else y + yi
    out_ref[...] = (base + y * gate).astype(out_ref.dtype)


@jax.jit
def pallas_sequential_preLN__mha_block_cached__moe_arch_mod__decode_kernel(
    A_x, A_k_cache, A_v_cache, A_wq, A_wo, B_x, B_w_r, B_w_gate, B_w_up, B_w_down,
):
    x2 = A_x.reshape(B, D)
    wr2 = B_w_r.reshape(D // 128, 128)
    kt = jnp.swapaxes(A_k_cache, 2, 3).reshape(NT, NROW, 8, S)
    vt = jnp.swapaxes(A_v_cache, 2, 3).reshape(NT, NROW, 8, S)

    any_spec = pl.BlockSpec(memory_space=pl.ANY)
    vmem_spec = pl.BlockSpec(memory_space=pltpu.VMEM)

    out = pl.pallas_call(
        _kernel,
        out_shape=jax.ShapeDtypeStruct((B, D), bf16),
        in_specs=[any_spec] * 9,
        out_specs=vmem_spec,
        scratch_shapes=[
            pltpu.VMEM((NB, NROW, 8, S), bf16),
            pltpu.VMEM((NB, NROW, 8, S), bf16),
            pltpu.VMEM((B, D), bf16),
            pltpu.VMEM((D // 128, 128), bf16),
            pltpu.VMEM((D, H * DH), bf16),
            pltpu.VMEM((H * DH, D), bf16),
            pltpu.VMEM((D, F), bf16),
            pltpu.VMEM((D, F), bf16),
            pltpu.VMEM((F, D), bf16),
            pltpu.VMEM((H, B, DH), f32),
            pltpu.VMEM((1, S), f32),
            pltpu.VMEM((B, 8, D), f32),
            pltpu.SemaphoreType.DMA((NB,)),
            pltpu.SemaphoreType.DMA((NB,)),
            pltpu.SemaphoreType.DMA((6,)),
            pltpu.SemaphoreType.DMA((NWD,)),
        ],
        compiler_params=pltpu.CompilerParams(vmem_limit_bytes=100 * 1024 * 1024,
                                             disable_bounds_checks=True),
    )(x2, wr2, kt, vt, A_wq, A_wo, B_w_gate, B_w_up, B_w_down)
    return out.reshape(B, 1, D)
```

```python
import jax
import jax.numpy as jnp
from jax import lax
import jax.experimental.pallas as pl
import jax.experimental.pallas.tpu as pltpu

B, H, S, DH, D, F = 4, 32, 8192, 192, 640, 1536
NT = B * H
EPS = 1e-5
SCALE = DH ** -0.5

NB = 3
WK = 512
WV = 256
NROW = DH // 8
NG = 6
RPG = NROW // NG
CB = S // 256
GU = RPG * CB
PW = 2
NDESC = GU // PW
DPI = NDESC // 32
NWD = 3

f32 = jnp.float32
bf16 = jnp.bfloat16


def _layernorm(x):
    m = jnp.mean(x, axis=-1, keepdims=True)
    c = x - m
    v = jnp.mean(c * c, axis=-1, keepdims=True)
    return c / jnp.sqrt(v + EPS)


def _kernel(x_hbm, wr_hbm, kt_hbm, vt_hbm, wq_hbm, wo_hbm, wg_hbm, wu_hbm, wd_hbm,
            out_ref,
            kbuf, vbuf, x_v, wr_v, wq_v, wo_v, wg_v, wu_v, wd_v,
            q_scr, s_scr, attn_scr,
            ksem, vsem, wsem, dsem):

    def issue(t, slot, c):
        for u in range(DPI):
            j = pl.multiple_of((c * DPI + u) * PW, PW)
            pltpu.make_async_copy(kt_hbm.at[t, :, pl.ds(j, PW)], kbuf.at[slot, :, pl.ds(j, PW)],
                                  ksem.at[slot]).start(priority=0)
            pltpu.make_async_copy(vt_hbm.at[t, :, pl.ds(j, PW)], vbuf.at[slot, :, pl.ds(j, PW)],
                                  vsem.at[slot]).start(priority=1)

    def wait_all(buf, sem):
        pltpu.make_async_copy(buf, buf, sem).wait()

    def rows_piece(hbm, vm, sem, r0, nrows, prio):
        pltpu.make_async_copy(hbm.at[pl.ds(r0, nrows), :], vm.at[pl.ds(r0, nrows), :], sem).start(priority=prio)

    def wq_go(r, _):
        r0 = pl.multiple_of(r * 8, 8)
        for u in range(2):
            c0 = u * (H * DH // 2)
            pltpu.make_async_copy(wq_hbm.at[pl.ds(r0, 8), pl.ds(c0, H * DH // 2)],
                                  wq_v.at[pl.ds(r0, 8), pl.ds(c0, H * DH // 2)], wsem.at[0]).start(priority=u)
        return 0
    lax.fori_loop(0, D // 8, wq_go, 0)

    x_copy = pltpu.make_async_copy(x_hbm, x_v, wsem.at[4])
    wr_copy = pltpu.make_async_copy(wr_hbm, wr_v, wsem.at[5])
    x_copy.start()
    wr_copy.start(priority=1)

    for i in range(NB - 1):
        def go(j, _):
            issue(i, i, j)
            return 0
        lax.fori_loop(0, 32, go, 0)

    def wo_go(r, _):
        for u in range(2):
            rows_piece(wo_hbm, wo_v, wsem.at[1], pl.multiple_of((2 * r + u) * 32, 32), 32, u)
        return 0
    lax.fori_loop(0, H * DH // 64, wo_go, 0)

    x_copy.wait()
    x = x_v[...].astype(f32)
    xn = _layernorm(x).astype(bf16)
    wait_all(wq_v, wsem.at[0])
    q_all = jnp.dot(xn, wq_v[...], preferred_element_type=f32)
    q_all = q_all.astype(bf16).astype(f32) * SCALE
    for h in range(H):
        q_scr[h] = q_all[:, h * DH:(h + 1) * DH]
    attn_scr[...] = jnp.zeros(attn_scr.shape, f32)
    wait_all(wo_v, wsem.at[1])

    row = lax.broadcasted_iota(jnp.int32, (DH, DH), 0)
    col = lax.broadcasted_iota(jnp.int32, (DH, DH), 1)
    eye = row == col

    def ffn_issue(c):
        @pl.when(c < 20)
        def _():
            r0 = pl.multiple_of(c * 32, 32)
            rows_piece(wg_hbm, wg_v, wsem.at[2], r0, 16, 0)
            rows_piece(wu_hbm, wu_v, wsem.at[3], r0, 16, 1)
            rows_piece(wg_hbm, wg_v, wsem.at[2], r0 + 16, 16, 0)
            rows_piece(wu_hbm, wu_v, wsem.at[3], r0 + 16, 16, 1)
        @pl.when(c >= 20)
        def _():
            cc = c - 20
            r0 = pl.multiple_of(cc * 128, 128)
            sem = dsem.at[lax.div(cc, jnp.int32(12 // NWD))]
            for u in range(4):
                rows_piece(wd_hbm, wd_v, sem, r0 + 32 * u, 32, u % 2)

    def step(t, slot, prefetch):
        b = lax.shift_right_logical(t, 5)
        h = t & (H - 1)
        pslot = jnp.where(slot == 0, NB - 1, slot - 1)

        qrow = q_scr[h, pl.ds(b, 1), :]
        qcol = jnp.sum(jnp.where(eye, qrow, 0.0), axis=1, keepdims=True)
        qb = jnp.broadcast_to(qcol, (DH, 128))

        wait_all(kbuf.at[slot], ksem.at[slot])

        def k_body(c, _):
            off = pl.multiple_of(c * WK, WK)
            for j in range(WK // 256):
                o2 = pl.multiple_of(off + j * 256, 256)
                cb = c * (WK // 256) + j
                parts = [[None] * 2 for _ in range(2)]
                for r in range(NROW):
                    kc = kbuf[slot, r // RPG, (r % RPG) * CB + cb].astype(f32)
                    qr = qb[r * 8:(r + 1) * 8, :]
                    for hf in range(2):
                        pr = kc[:, hf * 128:(hf + 1) * 128] * qr
                        a = parts[hf][r % 2]
                        parts[hf][r % 2] = pr if a is None else a + pr
                for hf in range(2):
                    sv = parts[hf][0] + parts[hf][1]
                    s_scr[:, pl.ds(pl.multiple_of(o2 + hf * 128, 128), 128)] = jnp.sum(sv, axis=0, keepdims=True)
            return 0

        lax.fori_loop(0, S // WK, k_body, 0)

        s = s_scr[...]
        m = jnp.max(s, axis=1, keepdims=True)
        p = jnp.exp(s - m)
        l = jnp.sum(p, axis=1, keepdims=True)
        s_scr[...] = p

        wait_all(vbuf.at[slot], vsem.at[slot])

        def v_body(c, acc):
            off = pl.multiple_of(c * WV, WV)
            p0 = jnp.broadcast_to(s_scr[:, pl.ds(off, 128)], (8, 128))
            p1 = jnp.broadcast_to(s_scr[:, pl.ds(pl.multiple_of(off + 128, 128), 128)], (8, 128))
            new = []
            for r in range(NROW):
                vc = vbuf[slot, r // RPG, (r % RPG) * CB + c].astype(f32)
                new.append(acc[r] + vc[:, 0:128] * p0 + vc[:, 128:256] * p1)
            if prefetch == "kv":
                issue(t + NB - 1, pslot, c)
            elif prefetch == "ffn":
                ffn_issue(c)
            return tuple(new)

        acc = lax.fori_loop(0, S // WV, v_body, tuple(jnp.zeros((8, 128), f32) for _ in range(NROW)))
        acc = jnp.concatenate(acc, axis=0)

        o = jnp.sum(acc, axis=1, keepdims=True) / l
        o = o.astype(bf16).astype(f32)
        wo_h = wo_v[pl.ds(pl.multiple_of(h * DH, 16), DH), :].astype(f32)
        contrib = (wo_h * o).reshape(DH // 8, 8, D).sum(axis=0)
        attn_scr[b] = attn_scr[b] + contrib
        nslot = slot + 1
        return jnp.where(nslot == NB, 0, nslot)

    slot = lax.fori_loop(0, NT - NB + 1, lambda t, s: step(t, s, "kv"), jnp.int32(0))
    slot = step(jnp.int32(NT - NB + 1), slot, "ffn")
    lax.fori_loop(NT - NB + 2, NT, lambda t, s: step(t, s, None), slot)

    attn = jnp.sum(attn_scr[...], axis=1)
    hres = x + attn
    hn = _layernorm(hres)
    hn16 = hn.astype(bf16)
    wr_copy.wait()
    hnr = hn16.astype(f32)
    racc = hnr[:, 0:128] * wr_v[0:1, :].astype(f32)
    for i in range(1, D // 128):
        racc = racc + hnr[:, i * 128:(i + 1) * 128] * wr_v[i:i + 1, :].astype(f32)
    r = jnp.sum(racc, axis=1, keepdims=True)
    gate = jax.nn.sigmoid(r)
    base = hres + hn
    wait_all(wg_v, wsem.at[2])
    g = jnp.dot(hn16, wg_v[...], preferred_element_type=f32)
    wait_all(wu_v, wsem.at[3])
    u = jnp.dot(hn16, wu_v[...], preferred_element_type=f32)
    mid = (g * jax.nn.sigmoid(g) * u).astype(bf16)
    CH = F // NWD
    y = None
    for i in range(NWD):
        wait_all(wd_v.at[pl.ds(i * CH, CH), :], dsem.at[i])
        yi = jnp.dot(mid[:, i * CH:(i + 1) * CH], wd_v[i * CH:(i + 1) * CH, :], preferred_element_type=f32)
        y = yi if y is None else y + yi
    out_ref[...] = (base + y * gate).astype(out_ref.dtype)


@jax.jit
def pallas_sequential_preLN__mha_block_cached__moe_arch_mod__decode_kernel(
    A_x, A_k_cache, A_v_cache, A_wq, A_wo, B_x, B_w_r, B_w_gate, B_w_up, B_w_down,
):
    x2 = A_x.reshape(B, D)
    wr2 = B_w_r.reshape(D // 128, 128)
    def blocks(a):
        a = jnp.swapaxes(a, 2, 3).reshape(NT, NROW, 8, CB, 256)
        return a.transpose(0, 1, 3, 2, 4).reshape(NT, NG, GU, 8, 256)
    kt = blocks(A_k_cache)
    vt = blocks(A_v_cache)

    any_spec = pl.BlockSpec(memory_space=pl.ANY)
    vmem_spec = pl.BlockSpec(memory_space=pltpu.VMEM)

    out = pl.pallas_call(
        _kernel,
        out_shape=jax.ShapeDtypeStruct((B, D), bf16),
        in_specs=[any_spec] * 9,
        out_specs=vmem_spec,
        scratch_shapes=[
            pltpu.VMEM((NB, NG, GU, 8, 256), bf16),
            pltpu.VMEM((NB, NG, GU, 8, 256), bf16),
            pltpu.VMEM((B, D), bf16),
            pltpu.VMEM((D // 128, 128), bf16),
            pltpu.VMEM((D, H * DH), bf16),
            pltpu.VMEM((H * DH, D), bf16),
            pltpu.VMEM((D, F), bf16),
            pltpu.VMEM((D, F), bf16),
            pltpu.VMEM((F, D), bf16),
            pltpu.VMEM((H, B, DH), f32),
            pltpu.VMEM((1, S), f32),
            pltpu.VMEM((B, 8, D), f32),
            pltpu.SemaphoreType.DMA((NB,)),
            pltpu.SemaphoreType.DMA((NB,)),
            pltpu.SemaphoreType.DMA((6,)),
            pltpu.SemaphoreType.DMA((NWD,)),
        ],
        compiler_params=pltpu.CompilerParams(vmem_limit_bytes=100 * 1024 * 1024,
                                             disable_bounds_checks=True),
    )(x2, wr2, kt, vt, A_wq, A_wo, B_w_gate, B_w_up, B_w_down)
    return out.reshape(B, 1, D)
```

```python
import jax
import jax.numpy as jnp
from jax import lax
import jax.experimental.pallas as pl
import jax.experimental.pallas.tpu as pltpu

B, H, S, DH, D, F = 4, 32, 8192, 192, 640, 1536
NT = B * H
EPS = 1e-5
SCALE = DH ** -0.5

NB = 3
NP = NT // 2
WV = 256
NROW = DH // 8
CB = S // 256
NG = 6
GU = 2 * NROW * CB // NG
RPG = GU // CB
PW = 2
NDESC = GU // PW
DPH = NDESC // 2
LAG = 32
OFF = NDESC + LAG
NWD = 3
NCH = 2
QCH = 8

f32 = jnp.float32
bf16 = jnp.bfloat16


def _layernorm(x):
    m = jnp.mean(x, axis=-1, keepdims=True)
    c = x - m
    v = jnp.mean(c * c, axis=-1, keepdims=True)
    return c / jnp.sqrt(v + EPS)


def _kernel(x_hbm, wr_hbm, kt_hbm, vt_hbm, wq_hbm, wo_hbm, wg_hbm, wu_hbm, wd_hbm,
            out_ref,
            kbuf, vbuf, x_v, wr_v, wq_v, wo_v, wg_v, wu_v, wd_v,
            q_scr, s_scr, attn_scr,
            ksem, vsem, wsem, dsem):

    def kv_issue(g):
        p = lax.shift_right_logical(g, 7)
        slot = lax.rem(p, NB)
        j = pl.multiple_of((g & (NDESC - 1)) * PW, PW)
        pltpu.make_async_copy(kt_hbm.at[p, :, pl.ds(j, PW)], kbuf.at[slot, :, pl.ds(j, PW)],
                              ksem.at[slot]).start(priority=0)
        pltpu.make_async_copy(vt_hbm.at[p, :, pl.ds(j, PW)], vbuf.at[slot, :, pl.ds(j, PW)],
                              vsem.at[slot]).start(priority=1)

    def wait_all(buf, sem):
        pltpu.make_async_copy(buf, buf, sem).wait()

    def rows_piece(hbm, vm, sem, r0, nrows, prio):
        pltpu.make_async_copy(hbm.at[pl.ds(r0, nrows), :], vm.at[pl.ds(r0, nrows), :], sem).start(priority=prio)

    def ffn_issue(i):
        @pl.when(i < 40)
        def _():
            r0 = pl.multiple_of(i * 16, 16)
            rows_piece(wg_hbm, wg_v, wsem.at[2], r0, 16, 0)
            rows_piece(wu_hbm, wu_v, wsem.at[3], r0, 16, 1)
        @pl.when(i >= 40)
        def _():
            ii = i - 40
            r0 = pl.multiple_of(ii * 64, 64)
            sem = dsem.at[lax.shift_right_logical(ii, 3)]
            rows_piece(wd_hbm, wd_v, sem, r0, 32, 0)
            rows_piece(wd_hbm, wd_v, sem, r0 + 32, 32, 1)

    x_copy = pltpu.make_async_copy(x_hbm, x_v, wsem.at[4])
    wr_copy = pltpu.make_async_copy(wr_hbm, wr_v, wsem.at[5])
    x_copy.start()
    wr_copy.start(priority=1)

    def wq_go(r, _):
        r0 = pl.multiple_of(r * 8, 8)
        for u in range(2):
            c0 = u * (H * DH // 2)
            pltpu.make_async_copy(wq_hbm.at[pl.ds(r0, 8), pl.ds(c0, H * DH // 2)],
                                  wq_v.at[pl.ds(r0, 8), pl.ds(c0, H * DH // 2)], wsem.at[0]).start(priority=u)
        return 0
    lax.fori_loop(0, D // 8, wq_go, 0)

    def pre(g, _):
        kv_issue(g)
        return 0
    lax.fori_loop(0, OFF, pre, 0)

    x_copy.wait()
    x = x_v[...].astype(f32)
    xn = _layernorm(x).astype(bf16)
    wait_all(wq_v, wsem.at[0])
    QW = H * DH // QCH
    WO_PER = H * DH // 64 // QCH
    for i in range(QCH):
        qc = jnp.dot(xn, wq_v[:, i * QW:(i + 1) * QW], preferred_element_type=f32)
        qc = qc.astype(bf16).astype(f32) * SCALE
        for hh in range(H // QCH):
            q_scr[i * (H // QCH) + hh] = qc[:, hh * DH:(hh + 1) * DH]

        def wo_go(r, _):
            for u in range(2):
                rows_piece(wo_hbm, wo_v, wsem.at[1], pl.multiple_of((2 * r + u) * 32, 32), 32, u)
            return 0
        lax.fori_loop(i * WO_PER, (i + 1) * WO_PER, wo_go, 0)
    attn_scr[...] = jnp.zeros(attn_scr.shape, f32)

    row = lax.broadcasted_iota(jnp.int32, (DH, DH), 0)
    col = lax.broadcasted_iota(jnp.int32, (DH, DH), 1)
    eye = row == col

    def step(t, k_issue, v_issue, first=False):
        b = lax.shift_right_logical(t, 5)
        h = t & (H - 1)
        hh = t & 1
        slot = lax.rem(lax.shift_right_logical(t, 1), NB)
        g0 = hh * (NG // 2)

        qrow = q_scr[h, pl.ds(b, 1), :]
        qcol = jnp.sum(jnp.where(eye, qrow, 0.0), axis=1, keepdims=True)
        qb = jnp.broadcast_to(qcol, (DH, 128))

        @pl.when(hh == 0)
        def _():
            wait_all(kbuf.at[slot], ksem.at[slot])

        def k_body(c, mx):
            off = pl.multiple_of(c * 256, 256)
            parts = [[None] * NCH for _ in range(2)]
            for r in range(NROW):
                kc = kbuf[slot, g0 + r // RPG, (r % RPG) * CB + c].astype(f32)
                qr = qb[r * 8:(r + 1) * 8, :]
                for hf in range(2):
                    pr = kc[:, hf * 128:(hf + 1) * 128] * qr
                    a_ = parts[hf][r % NCH]
                    parts[hf][r % NCH] = pr if a_ is None else a_ + pr
            for hf in range(2):
                sv = parts[hf][0]
                for i in range(1, NCH):
                    sv = sv + parts[hf][i]
                sv = sv + pltpu.roll(sv, 4, 0)
                sv = sv + pltpu.roll(sv, 2, 0)
                sv = sv + pltpu.roll(sv, 1, 0)
                s_scr[:, pl.ds(pl.multiple_of(off + hf * 128, 128), 128)] = sv
                mx = jnp.maximum(mx, sv)
            k_issue(c)
            return mx

        mx = lax.fori_loop(0, CB, k_body, jnp.full((8, 128), -jnp.inf, f32))
        m = jnp.max(mx, axis=1, keepdims=True)
        p = jnp.exp(s_scr[...] - m)
        l = jnp.sum(p, axis=1, keepdims=True)[0:1]
        s_scr[...] = p

        @pl.when(hh == 0)
        def _():
            wait_all(vbuf.at[slot], vsem.at[slot])

        def v_body(c, acc):
            off = pl.multiple_of(c * WV, WV)
            p0 = s_scr[:, pl.ds(off, 128)]
            p1 = s_scr[:, pl.ds(pl.multiple_of(off + 128, 128), 128)]
            new = []
            for r in range(NROW):
                vc = vbuf[slot, g0 + r // RPG, (r % RPG) * CB + c].astype(f32)
                new.append(acc[r] + vc[:, 0:128] * p0 + vc[:, 128:256] * p1)
            v_issue(c)
            return tuple(new)

        acc = lax.fori_loop(0, S // WV, v_body, tuple(jnp.zeros((8, 128), f32) for _ in range(NROW)))
        acc = jnp.concatenate(acc, axis=0)

        o = jnp.sum(acc, axis=1, keepdims=True) / l
        o = o.astype(bf16).astype(f32)

        @pl.when(t == 0)
        def _():
            wait_all(wo_v, wsem.at[1])

        wo_h = wo_v[pl.ds(pl.multiple_of(h * DH, 16), DH), :].astype(f32)
        contrib = (wo_h * o).reshape(DH // 8, 8, D).sum(axis=0)
        attn_scr[b] = attn_scr[b] + contrib

    def kv_k(t):
        def f(c):
            kv_issue(t * DPH + OFF + c)
        return f

    def kv_v(t):
        def f(c):
            kv_issue(t * DPH + OFF + DPH // 2 + c)
        return f

    def none(c):
        pass

    total = NP * NDESC
    n_full = (total - OFF) // DPH
    rem = (total - OFF) % DPH
    assert rem in (0, DPH // 2)

    def main(t, c):
        step(t, kv_k(t), kv_v(t))
        return c
    lax.fori_loop(0, n_full, main, 0)

    def ffn_all(base):
        def f(c):
            ffn_issue(base + c)
        return f

    def ffn_half(base):
        def f(c):
            @pl.when((c & 1) == 0)
            def _():
                ffn_issue(base + lax.shift_right_logical(c, 1))
        return f

    assert rem == DPH // 2 and n_full == NT - 3
    step(jnp.int32(NT - 3), kv_k(NT - 3), ffn_all(0))
    step(jnp.int32(NT - 2), none, ffn_half(32))
    step(jnp.int32(NT - 1), ffn_half(48), none)

    attn = jnp.sum(attn_scr[...], axis=1)
    hres = x + attn
    hn = _layernorm(hres)
    hn16 = hn.astype(bf16)
    wr_copy.wait()
    hnr = hn16.astype(f32)
    racc = hnr[:, 0:128] * wr_v[0:1, :].astype(f32)
    for i in range(1, D // 128):
        racc = racc + hnr[:, i * 128:(i + 1) * 128] * wr_v[i:i + 1, :].astype(f32)
    r = jnp.sum(racc, axis=1, keepdims=True)
    gate = jax.nn.sigmoid(r)
    base = hres + hn
    wait_all(wg_v, wsem.at[2])
    g = jnp.dot(hn16, wg_v[...], preferred_element_type=f32)
    wait_all(wu_v, wsem.at[3])
    u = jnp.dot(hn16, wu_v[...], preferred_element_type=f32)
    mid = (g * jax.nn.sigmoid(g) * u).astype(bf16)
    CH = F // NWD
    y = None
    for i in range(NWD):
        wait_all(wd_v.at[pl.ds(i * CH, CH), :], dsem.at[i])
        yi = jnp.dot(mid[:, i * CH:(i + 1) * CH], wd_v[i * CH:(i + 1) * CH, :], preferred_element_type=f32)
        y = yi if y is None else y + yi
    out_ref[...] = (base + y * gate).astype(out_ref.dtype)


@jax.jit
def pallas_sequential_preLN__mha_block_cached__moe_arch_mod__decode_kernel(
    A_x, A_k_cache, A_v_cache, A_wq, A_wo, B_x, B_w_r, B_w_gate, B_w_up, B_w_down,
):
    x2 = A_x.reshape(B, D)
    wr2 = B_w_r.reshape(D // 128, 128)

    def blocks(a):
        a = jnp.swapaxes(a, 2, 3).reshape(NT, NROW, 8, CB, 256)
        return a.transpose(0, 1, 3, 2, 4).reshape(NP, NG, GU, 8, 256)
    kt = blocks(A_k_cache)
    vt = blocks(A_v_cache)

    any_spec = pl.BlockSpec(memory_space=pl.ANY)
    vmem_spec = pl.BlockSpec(memory_space=pltpu.VMEM)

    out = pl.pallas_call(
        _kernel,
        out_shape=jax.ShapeDtypeStruct((B, D), bf16),
        in_specs=[any_spec] * 9,
        out_specs=vmem_spec,
        scratch_shapes=[
            pltpu.VMEM((NB, NG, GU, 8, 256), bf16),
            pltpu.VMEM((NB, NG, GU, 8, 256), bf16),
            pltpu.VMEM((B, D), bf16),
            pltpu.VMEM((D // 128, 128), bf16),
            pltpu.VMEM((D, H * DH), bf16),
            pltpu.VMEM((H * DH, D), bf16),
            pltpu.VMEM((D, F), bf16),
            pltpu.VMEM((D, F), bf16),
            pltpu.VMEM((F, D), bf16),
            pltpu.VMEM((H, B, DH), f32),
            pltpu.VMEM((8, S), f32),
            pltpu.VMEM((B, 8, D), f32),
            pltpu.SemaphoreType.DMA((NB,)),
            pltpu.SemaphoreType.DMA((NB,)),
            pltpu.SemaphoreType.DMA((6,)),
            pltpu.SemaphoreType.DMA((NWD,)),
        ],
        compiler_params=pltpu.CompilerParams(vmem_limit_bytes=100 * 1024 * 1024,
                                             disable_bounds_checks=True),
    )(x2, wr2, kt, vt, A_wq, A_wo, B_w_gate, B_w_up, B_w_down)
    return out.reshape(B, 1, D)
```

```python
import jax
import jax.numpy as jnp
from jax import lax
import jax.experimental.pallas as pl
import jax.experimental.pallas.tpu as pltpu

B, H, S, DH, D, F = 4, 32, 8192, 192, 640, 1536
NT = B * H
EPS = 1e-5
SCALE = DH ** -0.5

NB = 3
NP = NT // 2
NROW = DH // 8
CB = S // 256
NG = 6
GU = 2 * NROW * CB // NG
RPG = GU // CB
PW = 2
NDESC = GU // PW
LOG_NDESC = NDESC.bit_length() - 1
DPH = NDESC // 2
LAG = 32
OFF = NDESC + LAG
QCH = 8
NT1 = 16
WDCH = (512, 512, 512)

f32 = jnp.float32
bf16 = jnp.bfloat16


def _layernorm(x):
    m = jnp.mean(x, axis=-1, keepdims=True)
    c = x - m
    v = jnp.mean(c * c, axis=-1, keepdims=True)
    return c / jnp.sqrt(v + EPS)


def _kernel(x_hbm, wr_hbm, kt_hbm, vt_hbm, wq_hbm, wo_hbm, wg_hbm, wu_hbm, wd_hbm,
            out_ref,
            kbuf, vbuf, x_v, wr_v, wq_v, wo_v, wg_v, wu_v, wd_v,
            q_scr, s_scr, attn_scr,
            ksem, vsem, wsem, dsem):

    def kv_issue(g):
        p = lax.shift_right_logical(g, LOG_NDESC)
        slot = lax.rem(p, NB)
        j = pl.multiple_of((g & (NDESC - 1)) * PW, PW)
        pltpu.make_async_copy(kt_hbm.at[p, :, pl.ds(j, PW)], kbuf.at[slot, :, pl.ds(j, PW)],
                              ksem.at[slot]).start(priority=0)
        pltpu.make_async_copy(vt_hbm.at[p, :, pl.ds(j, PW)], vbuf.at[slot, :, pl.ds(j, PW)],
                              vsem.at[slot]).start(priority=1)

    def wait_all(buf, sem):
        pltpu.make_async_copy(buf, buf, sem).wait()

    def rows_piece(hbm, vm, sem, r0, nrows, prio):
        pltpu.make_async_copy(hbm.at[pl.ds(r0, nrows), :], vm.at[pl.ds(r0, nrows), :], sem).start(priority=prio)

    def ffn_issue(i):
        @pl.when(i < NT1)
        def _():
            r0 = pl.multiple_of(i * 16, 16)
            rows_piece(wg_hbm, wg_v, wsem.at[2], r0, 16, 1)
            rows_piece(wu_hbm, wu_v, wsem.at[3], r0, 16, 1)

        @pl.when(jnp.logical_and(i >= NT1, i < 40))
        def _():
            r0 = pl.multiple_of(i * 16, 16)
            rows_piece(wg_hbm, wg_v, wsem.at[2], r0, 16, 0)
            rows_piece(wu_hbm, wu_v, wsem.at[3], r0, 16, 1)

        @pl.when(i >= 40)
        def _():
            ii = i - 40
            r0 = pl.multiple_of(ii * 64, 64)
            ci = jnp.int32(0)
            edge = 0
            for w in WDCH[:-1]:
                edge += w // 64
                ci = ci + (ii >= edge).astype(jnp.int32)
            rows_piece(wd_hbm, wd_v, dsem.at[ci], r0, 32, 0)
            rows_piece(wd_hbm, wd_v, dsem.at[ci], r0 + 32, 32, 1)

    x_copy = pltpu.make_async_copy(x_hbm, x_v, wsem.at[4])
    wr_copy = pltpu.make_async_copy(wr_hbm, wr_v, wsem.at[5])
    x_copy.start()
    wr_copy.start(priority=1)

    def wq_go(r, c):
        r0 = pl.multiple_of(r * 8, 8)
        for u in range(2):
            c0 = u * (H * DH // 2)
            pltpu.make_async_copy(wq_hbm.at[pl.ds(r0, 8), pl.ds(c0, H * DH // 2)],
                                  wq_v.at[pl.ds(r0, 8), pl.ds(c0, H * DH // 2)], wsem.at[0]).start(priority=u)
        return c
    lax.fori_loop(0, D // 8, wq_go, 0)

    def pre(g, c):
        kv_issue(g)
        return c
    lax.fori_loop(0, OFF, pre, 0)

    x_copy.wait()
    x = x_v[...].astype(f32)
    xn = _layernorm(x).astype(bf16)
    wait_all(wq_v, wsem.at[0])
    qw = H * DH // QCH
    wo_per = H * DH // 64 // QCH
    for i in range(QCH):
        qc = jnp.dot(xn, wq_v[:, i * qw:(i + 1) * qw], preferred_element_type=f32)
        qc = qc.astype(bf16).astype(f32) * SCALE
        for hh in range(H // QCH):
            q_scr[i * (H // QCH) + hh] = qc[:, hh * DH:(hh + 1) * DH]

        def wo_go(r, c):
            for u in range(2):
                rows_piece(wo_hbm, wo_v, wsem.at[1], pl.multiple_of((2 * r + u) * 32, 32), 32, u)
            return c
        lax.fori_loop(i * wo_per, (i + 1) * wo_per, wo_go, 0)
    attn_scr[...] = jnp.zeros(attn_scr.shape, f32)

    row = lax.broadcasted_iota(jnp.int32, (DH, DH), 0)
    col = lax.broadcasted_iota(jnp.int32, (DH, DH), 1)
    eye = row == col

    def step(t, k_issue, v_issue):
        b = lax.shift_right_logical(t, 5)
        h = t & (H - 1)
        hh = t & 1
        slot = lax.rem(lax.shift_right_logical(t, 1), NB)
        g0 = hh * (NG // 2)

        qrow = q_scr[h, pl.ds(b, 1), :]
        qcol = jnp.sum(jnp.where(eye, qrow, 0.0), axis=1, keepdims=True)
        qb = jnp.broadcast_to(qcol, (DH, 128))

        @pl.when(hh == 0)
        def _():
            wait_all(kbuf.at[slot], ksem.at[slot])

        def k_body(c, mx):
            off = pl.multiple_of(c * 256, 256)
            parts = [[None] * 2 for _ in range(2)]
            for r in range(NROW):
                kc = kbuf[slot, g0 + r // RPG, (r % RPG) * CB + c].astype(f32)
                qr = qb[r * 8:(r + 1) * 8, :]
                for hf in range(2):
                    pr = kc[:, hf * 128:(hf + 1) * 128] * qr
                    prev = parts[hf][r % 2]
                    parts[hf][r % 2] = pr if prev is None else prev + pr
            for hf in range(2):
                sv = parts[hf][0] + parts[hf][1]
                sv = sv + pltpu.roll(sv, 4, 0)
                sv = sv + pltpu.roll(sv, 2, 0)
                sv = sv + pltpu.roll(sv, 1, 0)
                s_scr[:, pl.ds(pl.multiple_of(off + hf * 128, 128), 128)] = sv
                mx = jnp.maximum(mx, sv)
            k_issue(c)
            return mx

        mx = lax.fori_loop(0, CB, k_body, jnp.full((8, 128), -jnp.inf, f32))
        m = jnp.max(mx, axis=1, keepdims=True)
        p = jnp.exp(s_scr[...] - m)
        l = jnp.sum(p, axis=1, keepdims=True)[0:1]
        s_scr[...] = p

        @pl.when(hh == 0)
        def _():
            wait_all(vbuf.at[slot], vsem.at[slot])

        def v_body(c, acc):
            off = pl.multiple_of(c * 256, 256)
            p0 = s_scr[:, pl.ds(off, 128)]
            p1 = s_scr[:, pl.ds(pl.multiple_of(off + 128, 128), 128)]
            new = []
            for r in range(NROW):
                vc = vbuf[slot, g0 + r // RPG, (r % RPG) * CB + c].astype(f32)
                new.append(acc[r] + vc[:, 0:128] * p0 + vc[:, 128:256] * p1)
            v_issue(c)
            return tuple(new)

        acc = lax.fori_loop(0, CB, v_body, tuple(jnp.zeros((8, 128), f32) for _ in range(NROW)))
        acc = jnp.concatenate(acc, axis=0)
        o = jnp.sum(acc, axis=1, keepdims=True) / l
        o = o.astype(bf16).astype(f32)

        @pl.when(t == 0)
        def _():
            wait_all(wo_v, wsem.at[1])

        wo_h = wo_v[pl.ds(pl.multiple_of(h * DH, 16), DH), :].astype(f32)
        contrib = (wo_h * o).reshape(NROW, 8, D).sum(axis=0)
        attn_scr[b] = attn_scr[b] + contrib

    def kv_loop(t, phase):
        def f(c):
            kv_issue(t * DPH + OFF + phase * (DPH // 2) + c)
        return f

    def ffn_all(base):
        def f(c):
            ffn_issue(base + c)
        return f

    def ffn_half(base):
        def f(c):
            @pl.when((c & 1) == 0)
            def _():
                ffn_issue(base + lax.shift_right_logical(c, 1))
        return f

    def none(c):
        pass

    def main(t, c):
        step(t, kv_loop(t, 0), kv_loop(t, 1))
        return c
    lax.fori_loop(0, NT - 3, main, 0)

    assert (NT - 3) * DPH + OFF + DPH // 2 == NP * NDESC
    step(jnp.int32(NT - 3), kv_loop(NT - 3, 0), ffn_all(0))
    step(jnp.int32(NT - 2), none, ffn_half(32))
    step(jnp.int32(NT - 1), ffn_half(48), none)

    attn = jnp.sum(attn_scr[...], axis=1)
    hres = x + attn
    hn = _layernorm(hres)
    hn16 = hn.astype(bf16)
    wr_copy.wait()
    hnr = hn16.astype(f32)
    racc = hnr[:, 0:128] * wr_v[0:1, :].astype(f32)
    for i in range(1, D // 128):
        racc = racc + hnr[:, i * 128:(i + 1) * 128] * wr_v[i:i + 1, :].astype(f32)
    gate = jax.nn.sigmoid(jnp.sum(racc, axis=1, keepdims=True))
    base = hres + hn
    wait_all(wg_v, wsem.at[2])
    g = jnp.dot(hn16, wg_v[...], preferred_element_type=f32)
    wait_all(wu_v, wsem.at[3])
    u = jnp.dot(hn16, wu_v[...], preferred_element_type=f32)
    mid = (g * jax.nn.sigmoid(g) * u).astype(bf16)
    y = None
    r0 = 0
    for i, w in enumerate(WDCH):
        wait_all(wd_v.at[pl.ds(r0, w), :], dsem.at[i])
        yi = jnp.dot(mid[:, r0:r0 + w], wd_v[r0:r0 + w, :], preferred_element_type=f32)
        y = yi if y is None else y + yi
        r0 += w
    out_ref[...] = (base + y * gate).astype(out_ref.dtype)


@jax.jit
def pallas_sequential_preLN__mha_block_cached__moe_arch_mod__decode_kernel(
    A_x: jax.Array,
    A_k_cache: jax.Array,
    A_v_cache: jax.Array,
    A_wq: jax.Array,
    A_wo: jax.Array,
    B_x: jax.Array,
    B_w_r: jax.Array,
    B_w_gate: jax.Array,
    B_w_up: jax.Array,
    B_w_down: jax.Array,
):
    def blocks(a):
        a = jnp.swapaxes(a, 2, 3).reshape(NT, NROW, 8, CB, 256)
        return a.transpose(0, 1, 3, 2, 4).reshape(NP, NG, GU, 8, 256)

    any_spec = pl.BlockSpec(memory_space=pl.ANY)
    out = pl.pallas_call(
        _kernel,
        out_shape=jax.ShapeDtypeStruct((B, D), bf16),
        in_specs=[any_spec] * 9,
        out_specs=pl.BlockSpec(memory_space=pltpu.VMEM),
        scratch_shapes=[
            pltpu.VMEM((NB, NG, GU, 8, 256), bf16),
            pltpu.VMEM((NB, NG, GU, 8, 256), bf16),
            pltpu.VMEM((B, D), bf16),
            pltpu.VMEM((D // 128, 128), bf16),
            pltpu.VMEM((D, H * DH), bf16),
            pltpu.VMEM((H * DH, D), bf16),
            pltpu.VMEM((D, F), bf16),
            pltpu.VMEM((D, F), bf16),
            pltpu.VMEM((F, D), bf16),
            pltpu.VMEM((H, B, DH), f32),
            pltpu.VMEM((8, S), f32),
            pltpu.VMEM((B, 8, D), f32),
            pltpu.SemaphoreType.DMA((NB,)),
            pltpu.SemaphoreType.DMA((NB,)),
            pltpu.SemaphoreType.DMA((6,)),
            pltpu.SemaphoreType.DMA((len(WDCH),)),
        ],
        compiler_params=pltpu.CompilerParams(
            vmem_limit_bytes=100 * 1024 * 1024,
            disable_bounds_checks=True,
            disable_semaphore_checks=True,
        ),
    )(A_x.reshape(B, D), B_w_r.reshape(D // 128, 128), blocks(A_k_cache), blocks(A_v_cache),
      A_wq, A_wo, B_w_gate, B_w_up, B_w_down)
    return out.reshape(B, 1, D)
```

```python
import jax
import jax.numpy as jnp
from jax import lax
import jax.experimental.pallas as pl
import jax.experimental.pallas.tpu as pltpu

B, H, S, DH, D, F = 4, 32, 8192, 192, 640, 1536
NT = B * H
EPS = 1e-5
SCALE = DH ** -0.5

NB = 3
NP = NT // 2
NROW = DH // 8
CB = S // 256
NG = 6
GU = 2 * NROW * CB // NG
RPG = GU // CB
PW = 1
NDESC = GU // PW
LOG_NDESC = NDESC.bit_length() - 1
DPH = NDESC // 2
DPI = DPH // (2 * CB)
LAG = 32
OFF = NDESC + LAG
QCH = 8
NT1 = 16
WDCH = (512, 512, 512)

f32 = jnp.float32
bf16 = jnp.bfloat16


def _layernorm(x):
    m = jnp.mean(x, axis=-1, keepdims=True)
    c = x - m
    v = jnp.mean(c * c, axis=-1, keepdims=True)
    return c / jnp.sqrt(v + EPS)


def _kernel(x_hbm, wr_hbm, kt_hbm, vt_hbm, wq_hbm, wo_hbm, wg_hbm, wu_hbm, wd_hbm,
            out_ref,
            kbuf, vbuf, x_v, wr_v, wq_v, wo_v, wg_v, wu_v, wd_v,
            q_scr, s_scr, attn_scr,
            ksem, vsem, wsem, dsem):

    def kv_start(p, slot, j):
        j = pl.multiple_of(j * PW, PW)
        pltpu.make_async_copy(kt_hbm.at[p, :, pl.ds(j, PW)], kbuf.at[slot, :, pl.ds(j, PW)],
                              ksem.at[slot]).start(priority=0)
        pltpu.make_async_copy(vt_hbm.at[p, :, pl.ds(j, PW)], vbuf.at[slot, :, pl.ds(j, PW)],
                              vsem.at[slot]).start(priority=1)

    def kv_issue(g):
        p = lax.shift_right_logical(g, LOG_NDESC)
        kv_start(p, lax.rem(p, NB), g & (NDESC - 1))

    def kv_range(g0):
        p0 = lax.shift_right_logical(g0, LOG_NDESC)
        s0 = lax.rem(p0, NB)
        s1 = jnp.where(s0 == NB - 1, 0, s0 + 1)
        j0 = g0 & (NDESC - 1)

        def f(c):
            for u in range(DPI):
                jj = j0 + c * DPI + u
                wrap = jj >= NDESC
                kv_start(p0 + wrap.astype(jnp.int32), jnp.where(wrap, s1, s0), jj & (NDESC - 1))
        return f

    def wait_all(buf, sem):
        pltpu.make_async_copy(buf, buf, sem).wait()

    def rows_piece(hbm, vm, sem, r0, nrows, prio):
        pltpu.make_async_copy(hbm.at[pl.ds(r0, nrows), :], vm.at[pl.ds(r0, nrows), :], sem).start(priority=prio)

    def ffn_issue(i):
        @pl.when(i < NT1)
        def _():
            r0 = pl.multiple_of(i * 16, 16)
            rows_piece(wg_hbm, wg_v, wsem.at[2], r0, 16, 1)
            rows_piece(wu_hbm, wu_v, wsem.at[3], r0, 16, 1)

        @pl.when(jnp.logical_and(i >= NT1, i < 40))
        def _():
            r0 = pl.multiple_of(i * 16, 16)
            rows_piece(wg_hbm, wg_v, wsem.at[2], r0, 16, 0)
            rows_piece(wu_hbm, wu_v, wsem.at[3], r0, 16, 1)

        @pl.when(i >= 40)
        def _():
            ii = i - 40
            r0 = pl.multiple_of(ii * 64, 64)
            ci = jnp.int32(0)
            edge = 0
            for w in WDCH[:-1]:
                edge += w // 64
                ci = ci + (ii >= edge).astype(jnp.int32)
            rows_piece(wd_hbm, wd_v, dsem.at[ci], r0, 32, 0)
            rows_piece(wd_hbm, wd_v, dsem.at[ci], r0 + 32, 32, 1)

    x_copy = pltpu.make_async_copy(x_hbm, x_v, wsem.at[4])
    wr_copy = pltpu.make_async_copy(wr_hbm, wr_v, wsem.at[5])
    x_copy.start()
    wr_copy.start(priority=1)

    def wq_go(r, c):
        r0 = pl.multiple_of(r * 8, 8)
        for u in range(2):
            c0 = u * (H * DH // 2)
            pltpu.make_async_copy(wq_hbm.at[pl.ds(r0, 8), pl.ds(c0, H * DH // 2)],
                                  wq_v.at[pl.ds(r0, 8), pl.ds(c0, H * DH // 2)], wsem.at[0]).start(priority=u)
        return c
    lax.fori_loop(0, D // 8, wq_go, 0)

    def pre(g, c):
        kv_issue(g)
        return c
    lax.fori_loop(0, OFF, pre, 0)

    x_copy.wait()
    x = x_v[...].astype(f32)
    xn = _layernorm(x).astype(bf16)
    wait_all(wq_v, wsem.at[0])
    qw = H * DH // QCH
    wo_per = H * DH // 64 // QCH
    for i in range(QCH):
        qc = jnp.dot(xn, wq_v[:, i * qw:(i + 1) * qw], preferred_element_type=f32)
        qc = qc.astype(bf16).astype(f32) * SCALE
        for hh in range(H // QCH):
            q_scr[i * (H // QCH) + hh] = qc[:, hh * DH:(hh + 1) * DH]

        def wo_go(r, c):
            for u in range(2):
                rows_piece(wo_hbm, wo_v, wsem.at[1], pl.multiple_of((2 * r + u) * 32, 32), 32, u)
            return c
        lax.fori_loop(i * wo_per, (i + 1) * wo_per, wo_go, 0)
    attn_scr[...] = jnp.zeros(attn_scr.shape, f32)

    row = lax.broadcasted_iota(jnp.int32, (DH, DH), 0)
    col = lax.broadcasted_iota(jnp.int32, (DH, DH), 1)
    eye = row == col

    def step(t, k_issue, v_issue):
        b = lax.shift_right_logical(t, 5)
        h = t & (H - 1)
        hh = t & 1
        slot = lax.rem(lax.shift_right_logical(t, 1), NB)
        g0 = hh * (NG // 2)

        qrow = q_scr[h, pl.ds(b, 1), :]
        qcol = jnp.sum(jnp.where(eye, qrow, 0.0), axis=1, keepdims=True)
        qb = jnp.broadcast_to(qcol, (DH, 128))

        @pl.when(hh == 0)
        def _():
            wait_all(kbuf.at[slot], ksem.at[slot])

        def finalize(sv2, c, mx):
            off = pl.multiple_of(c * 256, 256)
            for hf in range(2):
                sv = sv2[hf]
                sv = sv + pltpu.roll(sv, 4, 0)
                sv = sv + pltpu.roll(sv, 2, 0)
                sv = sv + pltpu.roll(sv, 1, 0)
                s_scr[:, pl.ds(pl.multiple_of(off + hf * 128, 128), 128)] = sv
                mx = jnp.maximum(mx, sv)
            return mx

        def partials(c):
            parts = [[None] * 2 for _ in range(2)]
            for r in range(NROW):
                kc = kbuf[slot, g0 + r // RPG, (r % RPG) * CB + c].astype(f32)
                qr = qb[r * 8:(r + 1) * 8, :]
                for hf in range(2):
                    pr = kc[:, hf * 128:(hf + 1) * 128] * qr
                    prev = parts[hf][r % 2]
                    parts[hf][r % 2] = pr if prev is None else prev + pr
            return parts[0][0] + parts[0][1], parts[1][0] + parts[1][1]

        def k_body(c, carry):
            mx, lo, hi = carry
            new = partials(c)
            mx = finalize((lo, hi), jnp.maximum(c - 1, 0), mx)
            k_issue(c)
            return (mx,) + new

        ninf = jnp.full((8, 128), -jnp.inf, f32)
        mx, lo, hi = lax.fori_loop(0, CB, k_body, (ninf, ninf, ninf))
        mx = finalize((lo, hi), CB - 1, mx)
        m = jnp.max(mx, axis=1, keepdims=True)
        p = jnp.exp(s_scr[...] - m)
        l = jnp.sum(p, axis=1, keepdims=True)[0:1]
        s_scr[...] = p

        @pl.when(hh == 0)
        def _():
            wait_all(vbuf.at[slot], vsem.at[slot])

        def v_body(c, acc):
            off = pl.multiple_of(c * 256, 256)
            p0 = s_scr[:, pl.ds(off, 128)]
            p1 = s_scr[:, pl.ds(pl.multiple_of(off + 128, 128), 128)]
            new = []
            for r in range(NROW):
                vc = vbuf[slot, g0 + r // RPG, (r % RPG) * CB + c].astype(f32)
                new.append(acc[r] + (vc[:, 0:128] * p0 + vc[:, 128:256] * p1))
            v_issue(c)
            return tuple(new)

        acc = lax.fori_loop(0, CB, v_body, tuple(jnp.zeros((8, 128), f32) for _ in range(NROW)), unroll=2)
        acc = jnp.concatenate(acc, axis=0)
        o = jnp.sum(acc, axis=1, keepdims=True) / l
        o = o.astype(bf16).astype(f32)

        @pl.when(t == 0)
        def _():
            wait_all(wo_v, wsem.at[1])

        wo_h = wo_v[pl.ds(pl.multiple_of(h * DH, 16), DH), :].astype(f32)
        contrib = (wo_h * o).reshape(NROW, 8, D).sum(axis=0)
        attn_scr[b] = attn_scr[b] + contrib

    def kv_loop(t, phase):
        return kv_range(t * DPH + OFF + phase * (DPH // 2))

    def ffn_n(base, n, c0=0):
        span = CB - c0
        def f(c):
            cc = c - c0
            if n >= span:
                @pl.when(cc >= 0)
                def _():
                    for u in range(n // span):
                        ffn_issue(base + cc * (n // span) + u)
            else:
                sh = (span // n).bit_length() - 1
                @pl.when(jnp.logical_and(cc >= 0, (cc & ((1 << sh) - 1)) == 0))
                def _():
                    ffn_issue(base + lax.shift_right_logical(cc, sh))
        return f

    def none(c):
        pass

    def main(t, c):
        step(t, kv_loop(t, 0), kv_loop(t, 1))
        return c
    lax.fori_loop(0, NT - 3, main, 0)

    t3 = NT - 3
    nit = (NP * NDESC - (t3 * DPH + OFF + DPH // 2)) // DPI
    assert 0 <= nit < CB and (CB - nit) in (8, 16, 32)
    kv_last = kv_loop(jnp.int32(t3), 1)
    ffn_first = ffn_n(0, 32, nit)

    def t3_v_issue(c):
        if nit:
            @pl.when(c < nit)
            def _():
                kv_last(c)
        ffn_first(c)

    step(jnp.int32(t3), kv_loop(jnp.int32(t3), 0), t3_v_issue)
    step(jnp.int32(NT - 2), none, ffn_n(32, 16))
    step(jnp.int32(NT - 1), ffn_n(48, 16), none)

    attn = jnp.sum(attn_scr[...], axis=1)
    hres = x + attn
    hn = _layernorm(hres)
    hn16 = hn.astype(bf16)
    wr_copy.wait()
    hnr = hn16.astype(f32)
    racc = hnr[:, 0:128] * wr_v[0:1, :].astype(f32)
    for i in range(1, D // 128):
        racc = racc + hnr[:, i * 128:(i + 1) * 128] * wr_v[i:i + 1, :].astype(f32)
    gate = jax.nn.sigmoid(jnp.sum(racc, axis=1, keepdims=True))
    base = hres + hn
    wait_all(wg_v, wsem.at[2])
    g = jnp.dot(hn16, wg_v[...], preferred_element_type=f32)
    wait_all(wu_v, wsem.at[3])
    u = jnp.dot(hn16, wu_v[...], preferred_element_type=f32)
    mid = (g * jax.nn.sigmoid(g) * u).astype(bf16)
    y = None
    r0 = 0
    for i, w in enumerate(WDCH):
        wait_all(wd_v.at[pl.ds(r0, w), :], dsem.at[i])
        yi = jnp.dot(mid[:, r0:r0 + w], wd_v[r0:r0 + w, :], preferred_element_type=f32)
        y = yi if y is None else y + yi
        r0 += w
    out_ref[...] = (base + y * gate).astype(out_ref.dtype)


@jax.jit
def pallas_sequential_preLN__mha_block_cached__moe_arch_mod__decode_kernel(
    A_x: jax.Array,
    A_k_cache: jax.Array,
    A_v_cache: jax.Array,
    A_wq: jax.Array,
    A_wo: jax.Array,
    B_x: jax.Array,
    B_w_r: jax.Array,
    B_w_gate: jax.Array,
    B_w_up: jax.Array,
    B_w_down: jax.Array,
):
    def blocks(a):
        a = jnp.swapaxes(a, 2, 3).reshape(NT, NROW, 8, CB, 256)
        return a.transpose(0, 1, 3, 2, 4).reshape(NP, NG, GU, 8, 256)

    any_spec = pl.BlockSpec(memory_space=pl.ANY)
    out = pl.pallas_call(
        _kernel,
        out_shape=jax.ShapeDtypeStruct((B, D), bf16),
        in_specs=[any_spec] * 9,
        out_specs=pl.BlockSpec(memory_space=pltpu.VMEM),
        scratch_shapes=[
            pltpu.VMEM((NB, NG, GU, 8, 256), bf16),
            pltpu.VMEM((NB, NG, GU, 8, 256), bf16),
            pltpu.VMEM((B, D), bf16),
            pltpu.VMEM((D // 128, 128), bf16),
            pltpu.VMEM((D, H * DH), bf16),
            pltpu.VMEM((H * DH, D), bf16),
            pltpu.VMEM((D, F), bf16),
            pltpu.VMEM((D, F), bf16),
            pltpu.VMEM((F, D), bf16),
            pltpu.VMEM((H, B, DH), f32),
            pltpu.VMEM((8, S), f32),
            pltpu.VMEM((B, 8, D), f32),
            pltpu.SemaphoreType.DMA((NB,)),
            pltpu.SemaphoreType.DMA((NB,)),
            pltpu.SemaphoreType.DMA((6,)),
            pltpu.SemaphoreType.DMA((len(WDCH),)),
        ],
        compiler_params=pltpu.CompilerParams(
            vmem_limit_bytes=100 * 1024 * 1024,
            disable_bounds_checks=True,
            disable_semaphore_checks=True,
        ),
    )(A_x.reshape(B, D), B_w_r.reshape(D // 128, 128), blocks(A_k_cache), blocks(A_v_cache),
      A_wq, A_wo, B_w_gate, B_w_up, B_w_down)
    return out.reshape(B, 1, D)
```

```python
import jax
import jax.numpy as jnp
from jax import lax
import jax.experimental.pallas as pl
import jax.experimental.pallas.tpu as pltpu

B, H, S, DH, D, F = 4, 32, 8192, 192, 640, 1536
NT = B * H
EPS = 1e-5
SCALE = DH ** -0.5

NB = 3
NP = NT // 2
NROW = DH // 8
CB = S // 256
NG = 6
GU = 2 * NROW * CB // NG
RPG = GU // CB
PW = 1
NDESC = GU // PW
LOG_NDESC = NDESC.bit_length() - 1
DPH = NDESC // 2
DPI = DPH // (2 * CB)
LAG = 32
OFF = NDESC + LAG
QCH = 8
NT1 = 16
WDCH = (512, 512, 512)

f32 = jnp.float32
bf16 = jnp.bfloat16


def _layernorm(x):
    m = jnp.mean(x, axis=-1, keepdims=True)
    c = x - m
    v = jnp.mean(c * c, axis=-1, keepdims=True)
    return c / jnp.sqrt(v + EPS)


def _kernel(x_hbm, wr_hbm, kt_hbm, vt_hbm, wq_hbm, wo_hbm, wg_hbm, wu_hbm, wd_hbm,
            out_ref,
            kbuf, vbuf, x_v, wr_v, wq_v, wo_v, wg_v, wu_v, wd_v,
            q_scr, s_scr, attn_scr,
            ksem, vsem, wsem, dsem):

    def kv_start(p, slot, j):
        j = pl.multiple_of(j * PW, PW)
        pltpu.make_async_copy(kt_hbm.at[p, :, pl.ds(j, PW)], kbuf.at[slot, :, pl.ds(j, PW)],
                              ksem.at[slot]).start(priority=0)
        pltpu.make_async_copy(vt_hbm.at[p, :, pl.ds(j, PW)], vbuf.at[slot, :, pl.ds(j, PW)],
                              vsem.at[slot]).start(priority=1)

    def kv_issue(g):
        p = lax.shift_right_logical(g, LOG_NDESC)
        kv_start(p, lax.rem(p, NB), g & (NDESC - 1))

    def kv_range(g0):
        p0 = lax.shift_right_logical(g0, LOG_NDESC)
        s0 = lax.rem(p0, NB)
        s1 = jnp.where(s0 == NB - 1, 0, s0 + 1)
        j0 = g0 & (NDESC - 1)

        def f(c):
            for u in range(DPI):
                jj = j0 + c * DPI + u
                wrap = jj >= NDESC
                kv_start(p0 + wrap.astype(jnp.int32), jnp.where(wrap, s1, s0), jj & (NDESC - 1))
        return f

    def wait_all(buf, sem):
        pltpu.make_async_copy(buf, buf, sem).wait()

    def rows_piece(hbm, vm, sem, r0, nrows, prio):
        pltpu.make_async_copy(hbm.at[pl.ds(r0, nrows), :], vm.at[pl.ds(r0, nrows), :], sem).start(priority=prio)

    def ffn_issue(i):
        @pl.when(i < NT1)
        def _():
            r0 = pl.multiple_of(i * 16, 16)
            rows_piece(wg_hbm, wg_v, wsem.at[2], r0, 16, 1)
            rows_piece(wu_hbm, wu_v, wsem.at[3], r0, 16, 1)

        @pl.when(jnp.logical_and(i >= NT1, i < 40))
        def _():
            r0 = pl.multiple_of(i * 16, 16)
            rows_piece(wg_hbm, wg_v, wsem.at[2], r0, 16, 0)
            rows_piece(wu_hbm, wu_v, wsem.at[3], r0, 16, 1)

        @pl.when(i >= 40)
        def _():
            ii = i - 40
            r0 = pl.multiple_of(ii * 64, 64)
            ci = jnp.int32(0)
            edge = 0
            for w in WDCH[:-1]:
                edge += w // 64
                ci = ci + (ii >= edge).astype(jnp.int32)
            rows_piece(wd_hbm, wd_v, dsem.at[ci], r0, 32, 0)
            rows_piece(wd_hbm, wd_v, dsem.at[ci], r0 + 32, 32, 1)

    x_copy = pltpu.make_async_copy(x_hbm, x_v, wsem.at[4])
    wr_copy = pltpu.make_async_copy(wr_hbm, wr_v, wsem.at[5])
    x_copy.start()
    wr_copy.start(priority=1)

    def wq_go(r, c):
        r0 = pl.multiple_of(r * 8, 8)
        for u in range(2):
            c0 = u * (H * DH // 2)
            pltpu.make_async_copy(wq_hbm.at[pl.ds(r0, 8), pl.ds(c0, H * DH // 2)],
                                  wq_v.at[pl.ds(r0, 8), pl.ds(c0, H * DH // 2)], wsem.at[0]).start(priority=u)
        kv_issue(r)
        return c
    n_q = D // 8
    n_o = H * DH // 64
    assert n_q + n_o <= OFF
    lax.fori_loop(0, n_q, wq_go, 0)

    def pre(g, c):
        kv_issue(g)
        return c
    lax.fori_loop(n_q, OFF - n_o, pre, 0)

    x_copy.wait()
    x = x_v[...].astype(f32)
    xn = _layernorm(x).astype(bf16)
    wait_all(wq_v, wsem.at[0])
    qw = H * DH // QCH
    wo_per = n_o // QCH
    for i in range(QCH):
        qc = jnp.dot(xn, wq_v[:, i * qw:(i + 1) * qw], preferred_element_type=f32)
        qc = qc.astype(bf16).astype(f32) * SCALE
        for hh in range(H // QCH):
            q_scr[i * (H // QCH) + hh] = qc[:, hh * DH:(hh + 1) * DH]

        def wo_go(r, c):
            for u in range(2):
                rows_piece(wo_hbm, wo_v, wsem.at[1], pl.multiple_of((2 * r + u) * 32, 32), 32, u)
            kv_issue(OFF - n_o + r)
            return c
        lax.fori_loop(i * wo_per, (i + 1) * wo_per, wo_go, 0)
    attn_scr[...] = jnp.zeros(attn_scr.shape, f32)

    row = lax.broadcasted_iota(jnp.int32, (DH, DH), 0)
    col = lax.broadcasted_iota(jnp.int32, (DH, DH), 1)
    eye = row == col

    def step(t, k_issue, v_issue):
        b = lax.shift_right_logical(t, 5)
        h = t & (H - 1)
        hh = t & 1
        slot = lax.rem(lax.shift_right_logical(t, 1), NB)
        g0 = hh * (NG // 2)

        qrow = q_scr[h, pl.ds(b, 1), :]
        qcol = jnp.sum(jnp.where(eye, qrow, 0.0), axis=1, keepdims=True)
        qb = jnp.broadcast_to(qcol, (DH, 128))

        @pl.when(hh == 0)
        def _():
            wait_all(kbuf.at[slot], ksem.at[slot])

        def finalize(sv2, c, mx):
            off = pl.multiple_of(c * 256, 256)
            for hf in range(2):
                sv = sv2[hf]
                sv = sv + pltpu.roll(sv, 4, 0)
                sv = sv + pltpu.roll(sv, 2, 0)
                sv = sv + pltpu.roll(sv, 1, 0)
                s_scr[:, pl.ds(pl.multiple_of(off + hf * 128, 128), 128)] = sv
                mx = jnp.maximum(mx, sv)
            return mx

        def partials(c):
            parts = [[None] * 2 for _ in range(2)]
            for r in range(NROW):
                kc = kbuf[slot, g0 + r // RPG, (r % RPG) * CB + c].astype(f32)
                qr = qb[r * 8:(r + 1) * 8, :]
                for hf in range(2):
                    pr = kc[:, hf * 128:(hf + 1) * 128] * qr
                    prev = parts[hf][r % 2]
                    parts[hf][r % 2] = pr if prev is None else prev + pr
            return parts[0][0] + parts[0][1], parts[1][0] + parts[1][1]

        def k_body(c, carry):
            mx, lo, hi = carry
            new = partials(c)
            mx = finalize((lo, hi), jnp.maximum(c - 1, 0), mx)
            k_issue(c)
            return (mx,) + new

        ninf = jnp.full((8, 128), -jnp.inf, f32)
        mx, lo, hi = lax.fori_loop(0, CB, k_body, (ninf, ninf, ninf))
        mx = finalize((lo, hi), CB - 1, mx)
        m = jnp.max(mx, axis=1, keepdims=True)
        p = jnp.exp(s_scr[...] - m)
        l = jnp.sum(p, axis=1, keepdims=True)[0:1]
        s_scr[...] = p

        @pl.when(hh == 0)
        def _():
            wait_all(vbuf.at[slot], vsem.at[slot])

        def v_body(c, acc):
            off = pl.multiple_of(c * 256, 256)
            p0 = s_scr[:, pl.ds(off, 128)]
            p1 = s_scr[:, pl.ds(pl.multiple_of(off + 128, 128), 128)]
            new = []
            for r in range(NROW):
                vc = vbuf[slot, g0 + r // RPG, (r % RPG) * CB + c].astype(f32)
                new.append(acc[r] + (vc[:, 0:128] * p0 + vc[:, 128:256] * p1))
            v_issue(c)
            return tuple(new)

        acc = lax.fori_loop(0, CB, v_body, tuple(jnp.zeros((8, 128), f32) for _ in range(NROW)), unroll=2)
        acc = jnp.concatenate(acc, axis=0)
        o = jnp.sum(acc, axis=1, keepdims=True) / l
        o = o.astype(bf16).astype(f32)

        @pl.when(t == 0)
        def _():
            wait_all(wo_v, wsem.at[1])

        wo_h = wo_v[pl.ds(pl.multiple_of(h * DH, 16), DH), :].astype(f32)
        contrib = (wo_h * o).reshape(NROW, 8, D).sum(axis=0)
        attn_scr[b] = attn_scr[b] + contrib

    def kv_loop(t, phase):
        return kv_range(t * DPH + OFF + phase * (DPH // 2))

    def ffn_n(base, n, c0=0):
        span = CB - c0
        def f(c):
            cc = c - c0
            if n >= span:
                @pl.when(cc >= 0)
                def _():
                    for u in range(n // span):
                        ffn_issue(base + cc * (n // span) + u)
            else:
                sh = (span // n).bit_length() - 1
                @pl.when(jnp.logical_and(cc >= 0, (cc & ((1 << sh) - 1)) == 0))
                def _():
                    ffn_issue(base + lax.shift_right_logical(cc, sh))
        return f

    def none(c):
        pass

    def main(t, c):
        step(t, kv_loop(t, 0), kv_loop(t, 1))
        return c
    lax.fori_loop(0, NT - 3, main, 0)

    t3 = NT - 3
    nit = (NP * NDESC - (t3 * DPH + OFF + DPH // 2)) // DPI
    assert 0 <= nit < CB and (CB - nit) in (8, 16, 32)
    kv_last = kv_loop(jnp.int32(t3), 1)
    ffn_first = ffn_n(0, 32, nit)

    def t3_v_issue(c):
        if nit:
            @pl.when(c < nit)
            def _():
                kv_last(c)
        ffn_first(c)

    step(jnp.int32(t3), kv_loop(jnp.int32(t3), 0), t3_v_issue)
    step(jnp.int32(NT - 2), none, ffn_n(32, 16))
    step(jnp.int32(NT - 1), ffn_n(48, 16), none)

    attn = jnp.sum(attn_scr[...], axis=1)
    hres = x + attn
    hn = _layernorm(hres)
    hn16 = hn.astype(bf16)
    wr_copy.wait()
    hnr = hn16.astype(f32)
    racc = hnr[:, 0:128] * wr_v[0:1, :].astype(f32)
    for i in range(1, D // 128):
        racc = racc + hnr[:, i * 128:(i + 1) * 128] * wr_v[i:i + 1, :].astype(f32)
    gate = jax.nn.sigmoid(jnp.sum(racc, axis=1, keepdims=True))
    base = hres + hn
    wait_all(wg_v, wsem.at[2])
    g = jnp.dot(hn16, wg_v[...], preferred_element_type=f32)
    wait_all(wu_v, wsem.at[3])
    u = jnp.dot(hn16, wu_v[...], preferred_element_type=f32)
    mid = (g * jax.nn.sigmoid(g) * u).astype(bf16)
    y = None
    r0 = 0
    for i, w in enumerate(WDCH):
        wait_all(wd_v.at[pl.ds(r0, w), :], dsem.at[i])
        yi = jnp.dot(mid[:, r0:r0 + w], wd_v[r0:r0 + w, :], preferred_element_type=f32)
        y = yi if y is None else y + yi
        r0 += w
    out_ref[...] = (base + y * gate).astype(out_ref.dtype)


@jax.jit
def pallas_sequential_preLN__mha_block_cached__moe_arch_mod__decode_kernel(
    A_x: jax.Array,
    A_k_cache: jax.Array,
    A_v_cache: jax.Array,
    A_wq: jax.Array,
    A_wo: jax.Array,
    B_x: jax.Array,
    B_w_r: jax.Array,
    B_w_gate: jax.Array,
    B_w_up: jax.Array,
    B_w_down: jax.Array,
):
    def blocks(a):
        a = jnp.swapaxes(a, 2, 3).reshape(NT, NROW, 8, CB, 256)
        return a.transpose(0, 1, 3, 2, 4).reshape(NP, NG, GU, 8, 256)

    any_spec = pl.BlockSpec(memory_space=pl.ANY)
    out = pl.pallas_call(
        _kernel,
        out_shape=jax.ShapeDtypeStruct((B, D), bf16),
        in_specs=[any_spec] * 9,
        out_specs=pl.BlockSpec(memory_space=pltpu.VMEM),
        scratch_shapes=[
            pltpu.VMEM((NB, NG, GU, 8, 256), bf16),
            pltpu.VMEM((NB, NG, GU, 8, 256), bf16),
            pltpu.VMEM((B, D), bf16),
            pltpu.VMEM((D // 128, 128), bf16),
            pltpu.VMEM((D, H * DH), bf16),
            pltpu.VMEM((H * DH, D), bf16),
            pltpu.VMEM((D, F), bf16),
            pltpu.VMEM((D, F), bf16),
            pltpu.VMEM((F, D), bf16),
            pltpu.VMEM((H, B, DH), f32),
            pltpu.VMEM((8, S), f32),
            pltpu.VMEM((B, 8, D), f32),
            pltpu.SemaphoreType.DMA((NB,)),
            pltpu.SemaphoreType.DMA((NB,)),
            pltpu.SemaphoreType.DMA((6,)),
            pltpu.SemaphoreType.DMA((len(WDCH),)),
        ],
        compiler_params=pltpu.CompilerParams(
            vmem_limit_bytes=100 * 1024 * 1024,
            disable_bounds_checks=True,
            disable_semaphore_checks=True,
        ),
    )(A_x.reshape(B, D), B_w_r.reshape(D // 128, 128), blocks(A_k_cache), blocks(A_v_cache),
      A_wq, A_wo, B_w_gate, B_w_up, B_w_down)
    return out.reshape(B, 1, D)
```
